```python
import os as _os
_os.environ.setdefault("JAX_PLATFORMS", "cpu")
import jax
import jax.numpy as jnp

def _softmax(x, axis=-1):
    return jax.nn.softmax(x, axis=axis)
def _gelu(x):
    return jax.nn.gelu(x, approximate=True)
def _silu(x):
    return jax.nn.silu(x)
def _sigmoid(x):
    return jax.nn.sigmoid(x)
def _layernorm(x, axis=-1, eps=1e-5):
    m = jnp.mean(x, axis=axis, keepdims=True)
    v = jnp.var(x, axis=axis, keepdims=True)
    return (x - m) / jnp.sqrt(v + eps)
def _scatter_add(tgt, idx, src, axis=0):
    return tgt.at[idx].add(src)
def _segment_sum(src, seg, n):
    return jax.ops.segment_sum(src, seg, n)
class _Rng:
    def __init__(self, key):
        self._k = key
    def _next(self):
        self._k, sub = jax.random.split(self._k)
        return sub
    def normal(self, shape):
        return jax.random.normal(self._next(), shape, dtype=jnp.bfloat16)
    def randint(self, lo, hi, shape):
        return jax.random.randint(self._next(), shape, lo, hi, dtype=jnp.int32)
    def uniform(self, shape, lo=0.0, hi=1.0):
        return jax.random.uniform(self._next(), shape, jnp.bfloat16, lo, hi)
    def permutation(self, n):
        return jax.random.permutation(self._next(), n)


kernel_name = 'parallel_sum__grouped_kv_mqa__dense_activation_silu__prompt'

def setup_inputs():
    _rng = _Rng(jax.random.key(int.from_bytes(__import__("os").urandom(4), "little")))
    _w = (lambda a: (lambda t: t.astype(jnp.bfloat16) if jnp.issubdtype(t.dtype, jnp.floating) else t)(jnp.asarray(a)))
    def _A_setup():
        B, S, D, H = 1, 2048, 512, 32
        Dh = D // H
        return {
            "x": _w((lambda *s: _rng.normal(s) * 0.05)(B, S, D)),
            "wq": _w((lambda *s: _rng.normal(s) * 0.05)(D, H * Dh)),
            "wk": _w((lambda *s: _rng.normal(s) * 0.05)(D, Dh)),
            "wv": _w((lambda *s: _rng.normal(s) * 0.05)(D, Dh)),
            "wo": _w((lambda *s: _rng.normal(s) * 0.05)(H * Dh, D)),
        }
    _A_in = _A_setup()

    def _B_setup():
        B, S, D, F = 1, 2048, 512, 1376
        return {
            "x": _w((lambda *s: _rng.normal(s) * 0.05)(B, S, D)),
            "w1": _w((lambda *s: _rng.normal(s) * 0.05)(D, F) * (D ** -0.5)),
            "w2": _w((lambda *s: _rng.normal(s) * 0.05)(F, D) * (F ** -0.5)),
        }
    _B_in = _B_setup()

    return {
        "A_x": _A_in["x"],
        "A_wq": _A_in["wq"],
        "A_wk": _A_in["wk"],
        "A_wv": _A_in["wv"],
        "A_wo": _A_in["wo"],
        "B_x": _B_in["x"],
        "B_w1": _B_in["w1"],
        "B_w2": _B_in["w2"],
    }

def reference(A_x, A_wq, A_wk, A_wv, A_wo, B_x, B_w1, B_w2):
    def _A_ref(x, wq, wk, wv, wo):
        B, S, D = x.shape
        H = 32
        Dh = D // H
        q = (lambda x, *d: x.transpose(*d))((x @ wq).reshape(B, S, H, Dh), 0, 2, 1, 3)
        k = x @ wk
        v = x @ wv
        scores = jnp.einsum("bhqd,bkd->bhqk", q, k) * (Dh ** -0.5)
        p = _softmax(scores, axis=-1)
        o = jnp.einsum("bhqk,bkd->bhqd", p, v)
        return (lambda x, *d: x.transpose(*d))(o, 0, 2, 1, 3).reshape(B, S, H * Dh) @ wo

    def _B_ref(x, w1, w2):
        h = jnp.einsum("bsd,df->bsf", x, w1)
        h = _silu(h)
        out = jnp.einsum("bsf,fd->bsd", h, w2)
        return out

    x = A_x
    xn = _layernorm(x, axis=-1)
    return x + _A_ref(xn, A_wq, A_wk, A_wv, A_wo) + _B_ref(xn, B_w1, B_w2)
```

```python
import jax
import jax.numpy as jnp
import jax.experimental.pallas as pl
import jax.experimental.pallas.tpu as pltpu

S = 2048
D = 512
H = 32
DH = 16
TQ = 256
CK = 256
NC = S // CK
LOG2E = 1.4426950408889634
F32 = jnp.float32
BF16 = jnp.bfloat16


def _kernel(x_ref, wq_ref, wkv_ref, wo_ref, w1_ref, w2_ref, o_ref,
            xn_ref, k_ref, vt_ref, qt_ref, ot_ref, s0_ref, s1_ref):
    t = pl.program_id(0)

    @pl.when(t == 0)
    def _():
        for r in range(S // TQ):
            x = x_ref[r * TQ:(r + 1) * TQ, :].astype(F32)
            mean = jnp.mean(x, axis=-1, keepdims=True)
            xc = x - mean
            var = jnp.mean(xc * xc, axis=-1, keepdims=True)
            xn = (xc * jax.lax.rsqrt(var + 1e-5)).astype(BF16)
            xn_ref[r * TQ:(r + 1) * TQ, :] = xn
            kv = jnp.dot(xn, wkv_ref[...], preferred_element_type=F32)
            k_ref[r * TQ:(r + 1) * TQ, :] = kv[:, :DH].astype(BF16)
            vt_ref[:, r * TQ:(r + 1) * TQ] = kv.T[DH:2 * DH, :].astype(BF16)

    row = pl.multiple_of(t * TQ, TQ)
    xn = xn_ref[pl.ds(row, TQ), :]
    q = jnp.dot(xn, wq_ref[...], preferred_element_type=F32) * (DH ** -0.5 * LOG2E)
    qt_ref[...] = q.T.astype(BF16).reshape(H, DH, TQ)

    def qk_chunk(qt, s_ref, c, m):
        s = jnp.dot(k_ref[c * CK:(c + 1) * CK, :], qt, preferred_element_type=F32)
        s_ref[c * CK:(c + 1) * CK, :] = s
        mm = jnp.max(s.reshape(CK // 8, 8, TQ), axis=0)
        return mm if m is None else jnp.maximum(m, mm)

    def pv_chunk(s_ref, c, mb, l, o):
        s = s_ref[c * CK:(c + 1) * CK, :]
        p = jnp.exp2(s.reshape(CK // 8, 8, TQ) - mb[None])
        ll = jnp.sum(p, axis=0)
        oo = jnp.dot(vt_ref[:, c * CK:(c + 1) * CK], p.reshape(CK, TQ).astype(BF16),
                     preferred_element_type=F32)
        return (ll if l is None else l + ll), (oo if o is None else o + oo)

    def step(h, m_cur, s_cur, s_nxt):
        qt = qt_ref[jnp.minimum(h + 1, H - 1)]
        mb = jnp.broadcast_to(jnp.max(m_cur, axis=0, keepdims=True), (8, TQ))
        m = l = o = None
        for c in range(NC):
            m = qk_chunk(qt, s_nxt, c, m)
            l, o = pv_chunk(s_cur, c, mb, l, o)
        ot_ref[h] = (o / jnp.sum(l, axis=0, keepdims=True)).astype(BF16)
        return m

    m0 = None
    for c in range(NC):
        m0 = qk_chunk(qt_ref[0], s0_ref, c, m0)

    def body(i, m):
        m = step(2 * i, m, s0_ref, s1_ref)
        return step(2 * i + 1, m, s1_ref, s0_ref)

    jax.lax.fori_loop(0, H // 2, body, m0)

    attn = jax.lax.dot_general(ot_ref[...].reshape(H * DH, TQ), wo_ref[...],
                               (((0,), (0,)), ((), ())), preferred_element_type=F32)
    hid = jnp.dot(xn, w1_ref[...], preferred_element_type=F32)
    hid = (hid * jax.nn.sigmoid(hid)).astype(BF16)
    ffn = jnp.dot(hid, w2_ref[...], preferred_element_type=F32)
    o_ref[...] = (x_ref[pl.ds(row, TQ), :].astype(F32) + attn + ffn).astype(o_ref.dtype)


@jax.jit
def pallas_parallel_sum__grouped_kv_mqa__dense_activation_silu__prompt_kernel(
    A_x: jax.Array,
    A_wq: jax.Array,
    A_wk: jax.Array,
    A_wv: jax.Array,
    A_wo: jax.Array,
    B_x: jax.Array,
    B_w1: jax.Array,
    B_w2: jax.Array,
):
    del B_x
    F = B_w1.shape[1]
    wkv = jnp.pad(jnp.concatenate([A_wk, A_wv], axis=1), ((0, 0), (0, 128 - 2 * DH)))
    full = lambda shape: pl.BlockSpec(shape, lambda t: (0,) * len(shape))
    out = pl.pallas_call(
        _kernel,
        grid=(S // TQ,),
        in_specs=[full((S, D)), full((D, H * DH)), full((D, 128)), full((H * DH, D)),
                  full((D, F)), full((F, D))],
        out_specs=pl.BlockSpec((TQ, D), lambda t: (t, 0)),
        out_shape=jax.ShapeDtypeStruct((S, D), A_x.dtype),
        scratch_shapes=[
            pltpu.VMEM((S, D), BF16),
            pltpu.VMEM((S, DH), BF16),
            pltpu.VMEM((DH, S), BF16),
            pltpu.VMEM((H, DH, TQ), BF16),
            pltpu.VMEM((H, DH, TQ), BF16),
            pltpu.VMEM((S, TQ), F32),
            pltpu.VMEM((S, TQ), F32),
        ],
        compiler_params=pltpu.CompilerParams(
            dimension_semantics=("arbitrary",),
            vmem_limit_bytes=64 * 1024 * 1024,
        ),
    )(A_x.reshape(S, D), A_wq, wkv, A_wo, B_w1, B_w2)
    return out.reshape(A_x.shape)
```

```python
import jax
import jax.numpy as jnp
import jax.experimental.pallas as pl
import jax.experimental.pallas.tpu as pltpu

S = 2048
D = 512
H = 32
DH = 16
TQ = 256
NT = S // TQ
CK = 128
NC = S // CK
U = 8
DEP = 3
LAG = 4
OFF = 3
WAITS = {1: 2, 2: 5, 5: 8}
TR = 256
LOG2E = 1.4426950408889634
F32 = jnp.float32
BF16 = jnp.bfloat16
NT_DIMS = (((1,), (1,)), ((), ()))
TN_DIMS = (((0,), (0,)), ((), ()))


def _kernel(x_hbm, wq_hbm, wkt_hbm, wvt_hbm, wo_hbm, w1t_hbm, w2_hbm, o_hbm,
            x_ref, wq_ref, wkvt_ref, wo_ref, w1t_ref, w2_ref, out_ref,
            xn_ref, k_ref, vt_ref, qt_ref, ot_ref, s0_ref, s1_ref,
            x_sem, w_sem, o_sem):
    def x_copy(r):
        rows = pl.ds(r * TQ, TQ)
        return pltpu.make_async_copy(x_hbm.at[rows], x_ref.at[rows], x_sem.at[r])

    w_copies = [
        pltpu.make_async_copy(wkt_hbm, wkvt_ref.at[pl.ds(0, DH)], w_sem.at[0]),
        pltpu.make_async_copy(wvt_hbm, wkvt_ref.at[pl.ds(DH, DH)], w_sem.at[1]),
        pltpu.make_async_copy(wq_hbm, wq_ref, w_sem.at[2]),
        pltpu.make_async_copy(wo_hbm, wo_ref, w_sem.at[3]),
        pltpu.make_async_copy(w1t_hbm, w1t_ref, w_sem.at[4]),
        pltpu.make_async_copy(w2_hbm, w2_ref, w_sem.at[5]),
    ]
    x_copy(0).start()
    for c in w_copies[:3]:
        c.start()
    x_copy(1).start()

    def norm(r):
        rows = pl.ds(r * TQ, TQ)
        x = x_ref[rows, :].astype(F32)
        mean = jnp.mean(x, axis=-1, keepdims=True)
        xc = x - mean
        var = jnp.mean(xc * xc, axis=-1, keepdims=True)
        xn = (xc * jax.lax.rsqrt(var + 1e-5)).astype(BF16)
        xn_ref[rows, :] = xn
        return xn

    def proj(r, xn):
        rows = pl.ds(r * TQ, TQ)
        kvt = jax.lax.dot_general(wkvt_ref[...], xn, NT_DIMS, preferred_element_type=F32)
        k_ref[rows, :] = kvt.T[:, :DH].astype(BF16)
        vt_ref[r] = kvt[DH:, :].astype(BF16)
        q = jnp.dot(xn, wq_ref[...], preferred_element_type=F32) * (DH ** -0.5 * LOG2E)
        qt_ref[pl.ds(r * H, H)] = q.T.astype(BF16).reshape(H, DH, TQ)

    x_copy(0).wait()
    for r in range(2, NT):
        x_copy(r).start()
    norm(0)
    for c in w_copies[:3]:
        c.wait()
    for r in range(1, NT + 1):
        if r in WAITS:
            for r2 in range(r, WAITS[r]):
                x_copy(r2).wait()
            if WAITS[r] == NT:
                for c in w_copies[3:]:
                    c.start()
        if r < NT:
            norm(r)
        proj(r - 1, xn_ref[pl.ds((r - 1) * TQ, TQ), :])

    def qk_chunk(qt, s_ref, c, m):
        s = jnp.dot(k_ref[c * CK:(c + 1) * CK, :], qt, preferred_element_type=F32)
        s_ref[c * CK:(c + 1) * CK, :] = s
        mm = jnp.max(s.reshape(CK // 8, 8, TQ), axis=0)
        return mm if m is None else jnp.maximum(m, mm)

    def exp_chunk(s_ref, c, mb, l):
        s = s_ref[c * CK:(c + 1) * CK, :]
        p = jnp.exp2(s.reshape(CK // 8, 8, TQ) - mb[None])
        ll = jnp.sum(p, axis=0)
        return (ll if l is None else l + ll), p.reshape(CK, TQ).astype(BF16)

    def pv_chunk(p, c, o):
        r, off = divmod(c * CK, TQ)
        oo = jnp.dot(vt_ref[r, :, off:off + CK], p, preferred_element_type=F32)
        return oo if o is None else o + oo

    s_refs = (s0_ref, s1_ref)
    NU = NT * H

    def row_max(m):
        return jnp.broadcast_to(jnp.max(m, axis=0, keepdims=True), (8, TQ))

    m0 = m1 = None
    for c in range(NC):
        m0 = qk_chunk(qt_ref[0], s0_ref, c, m0)
    for c in range(OFF):
        m1 = qk_chunk(qt_ref[1], s1_ref, c, m1)

    def body(i, carry):
        mb0, m = carry
        mb = {0: mb0}
        ms, ps, ls = {}, {}, {}
        o = None
        for g in range(U * NC + LAG):
            if g < U * NC:
                j, c = divmod(g + OFF + NC, NC)
                qt = qt_ref[jnp.minimum(U * i + j, NU - 1)]
                ms[g] = m = qk_chunk(qt, s_refs[j % 2], c, m if c else None)
                if c == NC - 1:
                    mb[j] = row_max(m)
                j, c = divmod(g, NC)
                mbc = jnp.maximum(mb[j], jnp.minimum(mb[j], ms[g - DEP])) if g >= DEP else mb[j]
                ls[j], ps[g] = exp_chunk(s_refs[j % 2], c, mbc, ls.get(j))
            if g >= LAG:
                j, c = divmod(g - LAG, NC)
                o = pv_chunk(ps[g - LAG], c, o if c else None)
                if c == NC - 1:
                    ot_ref[U * i + j] = (o / jnp.sum(ls[j], axis=0, keepdims=True)).astype(BF16)
        return mb[U], m

    jax.lax.fori_loop(0, NU // U, body, (row_max(m0), m1))

    for c in w_copies[3:]:
        c.wait()

    def o_copy(r):
        rows = pl.ds(pl.multiple_of(r * TQ, TQ), TQ)
        return pltpu.make_async_copy(out_ref.at[rows], o_hbm.at[rows], o_sem.at[r])

    def dense(r, carry):
        rows = pl.ds(pl.multiple_of(r * TQ, TQ), TQ)
        hid = jax.lax.dot_general(xn_ref[rows, :], w1t_ref[...], NT_DIMS, preferred_element_type=F32)
        ot = ot_ref[pl.ds(r * H, H)].reshape(H * DH, TQ)
        attn = jax.lax.dot_general(ot, wo_ref[...], TN_DIMS, preferred_element_type=F32)
        hid = (hid * jax.nn.sigmoid(hid)).astype(BF16)
        ffn = jnp.dot(hid, w2_ref[...], preferred_element_type=F32)
        out_ref[rows, :] = (x_ref[rows, :].astype(F32) + attn + ffn).astype(out_ref.dtype)
        o_copy(r).start()
        return carry

    jax.lax.fori_loop(0, NT, dense, None, unroll=2)
    for r in range(NT):
        o_copy(r).wait()


@jax.jit
def pallas_parallel_sum__grouped_kv_mqa__dense_activation_silu__prompt_kernel(
    A_x: jax.Array,
    A_wq: jax.Array,
    A_wk: jax.Array,
    A_wv: jax.Array,
    A_wo: jax.Array,
    B_x: jax.Array,
    B_w1: jax.Array,
    B_w2: jax.Array,
):
    del B_x
    F = B_w1.shape[1]
    hbm = pl.BlockSpec(memory_space=pltpu.HBM)
    out = pl.pallas_call(
        _kernel,
        in_specs=[hbm] * 7,
        out_specs=hbm,
        out_shape=jax.ShapeDtypeStruct((S, D), A_x.dtype),
        scratch_shapes=[
            pltpu.VMEM((S, D), A_x.dtype),
            pltpu.VMEM((D, H * DH), BF16),
            pltpu.VMEM((2 * DH, D), BF16),
            pltpu.VMEM((H * DH, D), BF16),
            pltpu.VMEM((F, D), BF16),
            pltpu.VMEM((F, D), BF16),
            pltpu.VMEM((S, D), A_x.dtype),
            pltpu.VMEM((S, D), BF16),
            pltpu.VMEM((S, DH), BF16),
            pltpu.VMEM((NT, DH, TQ), BF16),
            pltpu.VMEM((NT * H, DH, TQ), BF16),
            pltpu.VMEM((NT * H, DH, TQ), BF16),
            pltpu.VMEM((S, TQ), F32),
            pltpu.VMEM((S, TQ), F32),
            pltpu.SemaphoreType.DMA((NT,)),
            pltpu.SemaphoreType.DMA((6,)),
            pltpu.SemaphoreType.DMA((NT,)),
        ],
        compiler_params=pltpu.CompilerParams(
            vmem_limit_bytes=64 * 1024 * 1024,
        ),
    )(A_x.reshape(S, D), A_wq, A_wk.T, A_wv.T, A_wo, B_w1.T, B_w2)
    return out.reshape(A_x.shape)
```
